```python
import jax
import jax.numpy as jnp

def _softmax(x, axis=-1):
    return jax.nn.softmax(x, axis=axis)
def _gelu(x):
    return jax.nn.gelu(x, approximate=True)
def _silu(x):
    return jax.nn.silu(x)
def _sigmoid(x):
    return jax.nn.sigmoid(x)
def _layernorm(x, axis=-1, eps=1e-5):
    m = jnp.mean(x, axis=axis, keepdims=True)
    v = jnp.var(x, axis=axis, keepdims=True)
    return (x - m) / jnp.sqrt(v + eps)
def _scatter_add(tgt, idx, src, axis=0):
    return tgt.at[idx].add(src)
def _segment_sum(src, seg, n):
    return jax.ops.segment_sum(src, seg, n)
class _Rng:
    def __init__(self, key):
        self._k = key
    def _next(self):
        self._k, sub = jax.random.split(self._k)
        return sub
    def normal(self, shape):
        return jax.random.normal(self._next(), shape, dtype=jnp.bfloat16)
    def randint(self, lo, hi, shape):
        return jax.random.randint(self._next(), shape, lo, hi, dtype=jnp.int32)
    def uniform(self, shape, lo=0.0, hi=1.0):
        return jax.random.uniform(self._next(), shape, jnp.bfloat16, lo, hi)
    def permutation(self, n):
        return jax.random.permutation(self._next(), n)


kernel_name = 'recurrent_scan__sliding_local_dilated__swiglu_ffn__prompt'

def setup_inputs():
    _rng = _Rng(jax.random.key(int.from_bytes(__import__("os").urandom(4), "little")))
    _w = (lambda a: (lambda t: t.astype(jnp.bfloat16) if jnp.issubdtype(t.dtype, jnp.floating) else t)(jnp.asarray(a)))
    def _A_setup():
        B, S, D = 1, 2048, 1024
        return {
            "x": _w((lambda *s: _rng.normal(s) * 0.05)(B, S, D)),
            "wqkv": _w((lambda *s: _rng.normal(s) * 0.05)(D, 3 * D)),
            "wo": _w((lambda *s: _rng.normal(s) * 0.05)(D, D)),
        }
    _A_in = _A_setup()

    def _B_setup():
        B, S, D, F = 1, 2048, 1024, 3584
        return {
            "x": _w((lambda *s: _rng.normal(s) * 0.05)(B, S, D)),
            "w_gate": _w((lambda *s: _rng.normal(s) * 0.05)(D, F)),
            "w_up": _w((lambda *s: _rng.normal(s) * 0.05)(D, F)),
            "w_down": _w((lambda *s: _rng.normal(s) * 0.05)(F, D)),
        }
    _B_in = _B_setup()

    return {
        "A_x": _A_in["x"],
        "A_wqkv": _A_in["wqkv"],
        "A_wo": _A_in["wo"],
        "B_x": _B_in["x"],
        "B_w_gate": _B_in["w_gate"],
        "B_w_up": _B_in["w_up"],
        "B_w_down": _B_in["w_down"],
    }

def reference(A_x, A_wqkv, A_wo, B_x, B_w_gate, B_w_up, B_w_down):
    def _A_ref(x, wqkv, wo):
        B, S, D = x.shape
        H = 32; Dh = D // H
        W, dil = 8, 2
        qkv = (lambda x, *d: x.transpose(*d))((x @ wqkv).reshape(B, S, 3, H, Dh), 2, 0, 3, 1, 4)
        q, k, v = qkv[0], qkv[1], qkv[2]
        scale = Dh ** -0.5
        pos = jnp.arange(S)
        off = jnp.arange(W) * dil
        idx = pos[:, None] - off[None, :]
        mask = idx >= 0
        idx_c = jnp.where(mask, idx, 0).reshape(-1)
        kg = k[:, :, idx_c, :].reshape(B, H, S, W, Dh)
        vg = v[:, :, idx_c, :].reshape(B, H, S, W, Dh)
        logits = jnp.einsum("bhsd,bhswd->bhsw", q, kg) * scale
        logits = jnp.where(mask[None, None, :, :], logits, -1e9)
        attn = _softmax(logits, axis=-1)
        o = jnp.einsum("bhsw,bhswd->bhsd", attn, vg)
        return (lambda x, *d: x.transpose(*d))(o, 0, 2, 1, 3).reshape(B, S, D) @ wo

    def _B_ref(x, w_gate, w_up, w_down):
        g = _silu(x @ w_gate)
        u = x @ w_up
        return (g * u) @ w_down

    x = A_x
    xn = _layernorm(x, axis=-1)
    s = _A_ref(xn, A_wqkv, A_wo)
    g = _silu(_B_ref(xn, B_w_gate, B_w_up, B_w_down))
    return x + s * g
```

```python
import jax
import jax.numpy as jnp
from jax import lax
import jax.experimental.pallas as pl
import jax.experimental.pallas.tpu as pltpu

S, D, F = 2048, 1024, 3584
H, DH, W, DIL = 32, 32, 8, 2
HALO = 16
NG = D // 128

TM = 512
TF = 896
QSEG = (0,512,1536,3072)
NT = S // TM
NF = F // TF


def _blk_transpose(arrs):
    shape = arrs[0].shape
    lane = lax.broadcasted_iota(jnp.int32, shape, 1)
    q = lane >> 2
    rolled = [arrs[0]] + [pltpu.roll(arrs[g], 4 * g, 1) for g in range(1, 8)]
    r = [rolled[(-m) % 8] for m in range(8)]
    for b in range(3):
        bit = (q & (1 << b)) != 0
        r = [jnp.where(bit, r[(j - (1 << b)) % 8], r[j]) for j in range(8)]
    return [r[0]] + [pltpu.roll(r[j], 128 - 4 * j, 1) for j in range(1, 8)]


def _attention_rows(q_s, k_s, v_s, att_s, r0, nrows, row_base):
    lane = lax.broadcasted_iota(jnp.int32, (16, 128), 1)
    even = (lane & 1) == 0
    low2 = (lane & 2) == 0
    scale = DH ** -0.5
    for rb in range(nrows // 16):
        r = r0 + rb * 16
        for ref in (k_s, v_s):
            t = _blk_transpose([ref[g, pl.ds(r + HALO, 16), :] for g in range(NG)])
            for g in range(NG):
                ref[g, pl.ds(r + HALO, 16), :] = t[g]
        qs = _blk_transpose([q_s[g, pl.ds(r, 16), :] for g in range(NG)])
        grow = row_base + r + lax.broadcasted_iota(jnp.int32, (16, 128), 0)
        logits = []
        for w in range(W):
            p = None
            for g in range(NG):
                t = qs[g] * k_s[g, pl.ds(r + HALO - DIL * w, 16), :]
                p = t if p is None else p + t
            y = p + jnp.where(even, pltpu.roll(p, 127, 1), pltpu.roll(p, 1, 1))
            z = y + jnp.where(low2, pltpu.roll(y, 126, 1), pltpu.roll(y, 2, 1))
            z = z * scale
            if w > 0:
                z = jnp.where(grow >= DIL * w, z, -1e9)
            logits.append(z)
        m = logits[0]
        for w in range(1, W):
            m = jnp.maximum(m, logits[w])
        es = [jnp.exp(l - m) for l in logits]
        den = es[0]
        for w in range(1, W):
            den = den + es[w]
        inv = pl.reciprocal(den, approx=False)
        ps = [e * inv for e in es]
        outs = []
        for g in range(NG):
            o = None
            for w in range(W):
                t = ps[w] * v_s[g, pl.ds(r + HALO - DIL * w, 16), :]
                o = t if o is None else o + t
            outs.append(pltpu.bitcast(o.astype(jnp.bfloat16), jnp.uint32))
        outs = _blk_transpose(outs)
        for g in range(NG):
            att_s[pl.ds(r, 16), g * 128:(g + 1) * 128] = pltpu.bitcast(outs[g], jnp.bfloat16)


def _layernorm(x):
    x = x.astype(jnp.float32)
    mean = jnp.mean(x, axis=-1, keepdims=True)
    xc = x - mean
    var = jnp.mean(xc * xc, axis=-1, keepdims=True)
    return (xc * lax.rsqrt(var + 1e-5)).astype(jnp.bfloat16)


def _kernel(x_hbm, wqkv_hbm, wo_hbm, wg_hbm, wu_hbm, wd_hbm, o_ref,
            x_s, wqkv_s, wo_s, wg_s, wu_s, wd_s,
            xn_s, xnn_s, q_s, k_s, v_s, att_s, acc_s,
            sem_x, sem_qkv, sem_o, sem_g, sem_u, sem_d):
    i = pl.program_id(0)

    def x_copy(t):
        return pltpu.make_async_copy(x_hbm.at[pl.ds(t * TM, TM), :], x_s.at[pl.ds(t * TM, TM), :], sem_x.at[t])

    def qkv_copy(t):
        c0, n = QSEG[t], QSEG[t + 1] - QSEG[t]
        return pltpu.make_async_copy(wqkv_hbm.at[:, pl.ds(c0, n)], wqkv_s.at[:, pl.ds(c0, n)], sem_qkv.at[t])

    def wo_copy():
        return pltpu.make_async_copy(wo_hbm, wo_s, sem_o.at[0])

    def g_copy(j):
        return pltpu.make_async_copy(wg_hbm.at[:, pl.ds(j * TF, TF)], wg_s.at[j], sem_g.at[j])

    def u_copy(j):
        return pltpu.make_async_copy(wu_hbm.at[:, pl.ds(j * TF, TF)], wu_s.at[j], sem_u.at[j])

    def d_copy(j):
        return pltpu.make_async_copy(wd_hbm.at[pl.ds(j * TF, TF), :], wd_s.at[j], sem_d.at[j])

    def ffn_start(j):
        g_copy(j).start()
        u_copy(j).start()
        d_copy(j).start()

    @pl.when(i == 0)
    def _():
        x_copy(0).start()
        qkv_copy(0).start()
        k_s[:, 0:HALO, :] = jnp.zeros((NG, HALO, 128), jnp.float32)
        v_s[:, 0:HALO, :] = jnp.zeros((NG, HALO, 128), jnp.float32)
        acc_s[...] = jnp.zeros_like(acc_s)
        x_copy(0).wait()
        xn_s[...] = _layernorm(x_s[0:TM, :])

    nxt = jnp.minimum(i + 1, NT - 1)
    rows_per = TM // NF
    nseg = len(QSEG) - 1

    for t in range(nseg):
        @pl.when(i == 0)
        def _():
            qkv_copy(t).wait()
            if t + 1 < nseg:
                qkv_copy(t + 1).start()
            else:
                ffn_start(0)
                x_copy(1).start()
        res = jnp.dot(xn_s[...], wqkv_s[:, QSEG[t]:QSEG[t + 1]], preferred_element_type=jnp.float32)
        for c in range(QSEG[t] // 128, QSEG[t + 1] // 128):
            dst, off = ((q_s, 0), (k_s, HALO), (v_s, HALO))[c // NG]
            lc = c * 128 - QSEG[t]
            dst[c % NG, off:off + TM, :] = res[:, lc:lc + 128]

    def ffn_body(j, c):
        @pl.when(i == 0)
        def _():
            g_copy(j).wait()
            u_copy(j).wait()
            d_copy(j).wait()

        @pl.when(jnp.logical_and(i < NT - 1, j == 0))
        def _():
            x_copy(nxt).wait()

        @pl.when(jnp.logical_and(i == 0, j == 0))
        def _():
            ffn_start(1)

        @pl.when(jnp.logical_and(i == 0, j == 1))
        def _():
            for jj in range(2, NF):
                ffn_start(jj)
            wo_copy().start()
            for t in range(2, NT):
                x_copy(t).start()

        xn = xn_s[...]
        g = jnp.dot(xn, wg_s[j], preferred_element_type=jnp.float32)
        u = jnp.dot(xn, wu_s[j], preferred_element_type=jnp.float32)
        h = (g * jax.nn.sigmoid(g) * u).astype(jnp.bfloat16)
        acc_s[...] += jnp.dot(h, wd_s[j], preferred_element_type=jnp.float32)
        r0 = pl.multiple_of(j * rows_per, 16)
        _attention_rows(q_s, k_s, v_s, att_s, r0, rows_per, i * TM)
        xr = pl.multiple_of(nxt * TM + r0, 16)
        xnn_s[pl.ds(r0, rows_per), :] = _layernorm(x_s[pl.ds(xr, rows_per), :])
        return c
    lax.fori_loop(0, NF, ffn_body, 0)

    @pl.when(i == 0)
    def _():
        wo_copy().wait()

    k_s[:, 0:HALO, :] = k_s[:, TM:TM + HALO, :]
    v_s[:, 0:HALO, :] = v_s[:, TM:TM + HALO, :]
    xn_s[...] = xnn_s[...]

    s = jnp.dot(att_s[...], wo_s[...], preferred_element_type=jnp.float32)
    f = acc_s[...]
    acc_s[...] = jnp.zeros_like(acc_s)
    xcur = x_s[pl.ds(pl.multiple_of(i * TM, TM), TM), :]
    o_ref[...] = (xcur.astype(jnp.float32) + s * (f * jax.nn.sigmoid(f))).astype(o_ref.dtype)


@jax.jit
def pallas_recurrent_scan__sliding_local_dilated__swiglu_ffn__prompt_kernel(
    A_x, A_wqkv, A_wo, B_x, B_w_gate, B_w_up, B_w_down):
    x = A_x.reshape(S, D)
    hbm = pl.BlockSpec(memory_space=pl.ANY)
    bf = jnp.bfloat16
    out = pl.pallas_call(
        _kernel,
        grid=(NT,),
        in_specs=[hbm] * 6,
        out_specs=pl.BlockSpec((TM, D), lambda i: (i, 0)),
        out_shape=jax.ShapeDtypeStruct((S, D), bf),
        scratch_shapes=[
            pltpu.VMEM((S, D), bf),
            pltpu.VMEM((D, 3 * D), bf),
            pltpu.VMEM((D, D), bf),
            pltpu.VMEM((NF, D, TF), bf),
            pltpu.VMEM((NF, D, TF), bf),
            pltpu.VMEM((NF, TF, D), bf),
            pltpu.VMEM((TM, D), bf),
            pltpu.VMEM((TM, D), bf),
            pltpu.VMEM((NG, TM, 128), jnp.float32),
            pltpu.VMEM((NG, TM + HALO, 128), jnp.float32),
            pltpu.VMEM((NG, TM + HALO, 128), jnp.float32),
            pltpu.VMEM((TM, D), bf),
            pltpu.VMEM((TM, D), jnp.float32),
            pltpu.SemaphoreType.DMA((NT,)),
            pltpu.SemaphoreType.DMA((len(QSEG) - 1,)),
            pltpu.SemaphoreType.DMA((1,)),
            pltpu.SemaphoreType.DMA((NF,)),
            pltpu.SemaphoreType.DMA((NF,)),
            pltpu.SemaphoreType.DMA((NF,)),
        ],
        compiler_params=pltpu.CompilerParams(
            dimension_semantics=("arbitrary",),
            vmem_limit_bytes=100 * 1024 * 1024,
        ),
    )(x, A_wqkv, A_wo, B_w_gate, B_w_up, B_w_down)
    return out.reshape(1, S, D)
```

```python
import jax
import jax.numpy as jnp
from jax import lax
import jax.experimental.pallas as pl
import jax.experimental.pallas.tpu as pltpu

S, D, F = 2048, 1024, 3584
H, DH, W, DIL = 32, 32, 8, 2
HALO = 16
NG = D // 128

TM = 512
TF = 896
NT = S // TM
NF = F // TF
NOC = 4
OC = D // NOC
XC = 4
XR = TM // XC
QA, NQA = 256, 2
QB, NQB = 512, 5

SEM_X0 = 0
SEM_X = SEM_X0 + XC
SEM_QA = SEM_X + NT
SEM_QB = SEM_QA + NQA
SEM_O = SEM_QB + NQB
SEM_G = SEM_O + 1
SEM_U = SEM_G + NF
SEM_D = SEM_U + NF
NSEM = SEM_D + NF


def _blk_transpose(arrs):
    shape = arrs[0].shape
    lane = lax.broadcasted_iota(jnp.int32, shape, 1)
    q = lane >> 2
    rolled = [arrs[0]] + [pltpu.roll(arrs[g], 4 * g, 1) for g in range(1, 8)]
    r = [rolled[(-m) % 8] for m in range(8)]
    for b in range(3):
        bit = (q & (1 << b)) != 0
        r = [jnp.where(bit, r[(j - (1 << b)) % 8], r[j]) for j in range(8)]
    return [r[0]] + [pltpu.roll(r[j], 128 - 4 * j, 1) for j in range(1, 8)]


def _attention_rows(qkv_s, att_s, r0, nrows, row_base, extra):
    lane = lax.broadcasted_iota(jnp.int32, (16, 128), 1)
    even = (lane & 1) == 0
    low2 = (lane & 2) == 0
    scale = DH ** -0.5
    for rb in range(nrows // 16):
        r = r0 + rb * 16
        for base in (NG, 2 * NG):
            t = _blk_transpose([qkv_s[base + g, pl.ds(r + HALO, 16), :] for g in range(NG)])
            for g in range(NG):
                qkv_s[base + g, pl.ds(r + HALO, 16), :] = t[g]
        qs = _blk_transpose([qkv_s[g, pl.ds(r + HALO, 16), :] for g in range(NG)])
        grow = row_base + r + lax.broadcasted_iota(jnp.int32, (16, 128), 0)
        logits = []
        for w in range(W):
            p = None
            for g in range(NG):
                t = qs[g] * qkv_s[NG + g, pl.ds(r + HALO - DIL * w, 16), :]
                p = t if p is None else p + t
            y = p + jnp.where(even, pltpu.roll(p, 127, 1), pltpu.roll(p, 1, 1))
            z = y + jnp.where(low2, pltpu.roll(y, 126, 1), pltpu.roll(y, 2, 1))
            z = z * scale
            if w > 0:
                z = jnp.where(grow >= DIL * w, z, -1e9)
            logits.append(z)
        m = logits[0]
        for w in range(1, W):
            m = jnp.maximum(m, logits[w])
        es = [jnp.exp(l - m) for l in logits]
        den = es[0]
        for w in range(1, W):
            den = den + es[w]
        inv = pl.reciprocal(den, approx=False)
        ps = [e * inv for e in es]
        outs = []
        for g in range(NG):
            o = None
            for w in range(W):
                t = ps[w] * qkv_s[2 * NG + g, pl.ds(r + HALO - DIL * w, 16), :]
                o = t if o is None else o + t
            outs.append(pltpu.bitcast(o.astype(jnp.bfloat16), jnp.uint32))
        outs = _blk_transpose(outs)
        for g in range(NG):
            att_s[pl.ds(r, 16), g * 128:(g + 1) * 128] = pltpu.bitcast(outs[g], jnp.bfloat16)
        extra(r)


def _silu(x):
    t = 0.5 * x
    return t + t * jnp.tanh(t)


def _layernorm(x):
    x = x.astype(jnp.float32)
    mean = jnp.mean(x, axis=-1, keepdims=True)
    xc = x - mean
    var = jnp.mean(xc * xc, axis=-1, keepdims=True)
    return (xc * lax.rsqrt(var + 1e-5)).astype(jnp.bfloat16)


def _kernel(x_hbm, wqkv_hbm, wo_hbm, wg_hbm, wu_hbm, wd_hbm, o_hbm,
            x_s, wqkv_s, wo_s, wg_s, wu_s, wd_s,
            xn_s, qkv_s, att_s, acc_s, o_s, sem, sem_out):
    i = pl.program_id(0)

    def x0_copy(c):
        return pltpu.make_async_copy(x_hbm.at[pl.ds(c * XR, XR), :], x_s.at[pl.ds(c * XR, XR), :], sem.at[SEM_X0 + c])

    def x_copy(t):
        return pltpu.make_async_copy(x_hbm.at[pl.ds(t * TM, TM), :], x_s.at[pl.ds(t * TM, TM), :], sem.at[SEM_X + t])

    def qa_copy(t):
        return pltpu.make_async_copy(wqkv_hbm.at[:, pl.ds(t * QA, QA)], wqkv_s.at[:, pl.ds(t * QA, QA)], sem.at[SEM_QA + t])

    def qb_copy(t):
        c0 = NQA * QA + t * QB
        return pltpu.make_async_copy(wqkv_hbm.at[:, pl.ds(c0, QB)], wqkv_s.at[:, pl.ds(c0, QB)], sem.at[SEM_QB + t])

    def wo_copy():
        return pltpu.make_async_copy(wo_hbm, wo_s, sem.at[SEM_O])

    def g_copy(j):
        return pltpu.make_async_copy(wg_hbm.at[:, pl.ds(j * TF, TF)], wg_s.at[j], sem.at[SEM_G + j])

    def u_copy(j):
        return pltpu.make_async_copy(wu_hbm.at[:, pl.ds(j * TF, TF)], wu_s.at[j], sem.at[SEM_U + j])

    def d_copy(j):
        return pltpu.make_async_copy(wd_hbm.at[pl.ds(j * TF, TF), :], wd_s.at[j], sem.at[SEM_D + j])

    def o_copy(t, c):
        return pltpu.make_async_copy(o_s.at[:, pl.ds(c * OC, OC)], o_hbm.at[pl.ds(t * TM, TM), pl.ds(c * OC, OC)], sem_out.at[c])

    def qkv_cols(xn, c0, n):
        static = isinstance(c0, int)
        w = wqkv_s[:, c0:c0 + n] if static else wqkv_s[:, pl.ds(pl.multiple_of(c0, 128), n)]
        res = jnp.dot(xn, w, preferred_element_type=jnp.float32)
        g0 = c0 // 128
        for k in range(n // 128):
            qkv_s[g0 + k, HALO:HALO + TM, :] = res[:, k * 128:(k + 1) * 128]

    @pl.when(i == 0)
    def _():
        for c in range(XC):
            x0_copy(c).start()
        for t in range(NQA):
            qa_copy(t).start()
        for t in range(NQB):
            qb_copy(t).start()
        for jj in range(NF):
            g_copy(jj).start()
            u_copy(jj).start()
            d_copy(jj).start()
            if jj == 0:
                x_copy(1).start()
        wo_copy().start()
        for t in range(2, NT):
            x_copy(t).start()
        qkv_s[NG:3 * NG, 0:HALO, :] = jnp.zeros((2 * NG, HALO, 128), jnp.float32)

        def ln0(c, carry):
            r = pl.multiple_of(c * XR, XR)
            acc_s[pl.ds(r, XR), :] = jnp.zeros((XR, D), jnp.float32)
            x0_copy(c).wait()
            xn_s[0, pl.ds(r, XR), :] = _layernorm(x_s[pl.ds(r, XR), :])
            return carry
        lax.fori_loop(0, XC, ln0, 0)

        def qa_body(t, carry):
            qa_copy(t).wait()
            qkv_cols(xn_s[0], t * QA, QA)
            return carry
        lax.fori_loop(0, NQA, qa_body, 0)

        def qb_body(t, carry):
            qb_copy(t).wait()
            qkv_cols(xn_s[0], NQA * QA + t * QB, QB)
            return carry
        lax.fori_loop(0, NQB, qb_body, 0)

    nxt = jnp.minimum(i + 1, NT - 1)
    slot = i % 2
    rows_per = TM // NF

    def ffn_body(j, c):
        @pl.when(i == 0)
        def _():
            g_copy(j).wait()
            u_copy(j).wait()
            d_copy(j).wait()

        @pl.when(jnp.logical_and(i < NT - 1, j == 0))
        def _():
            x_copy(nxt).wait()

        xn = xn_s[slot]
        g = jnp.dot(xn, wg_s[j], preferred_element_type=jnp.float32)
        u = jnp.dot(xn, wu_s[j], preferred_element_type=jnp.float32)
        h = (_silu(g) * u).astype(jnp.bfloat16)
        acc_s[...] += jnp.dot(h, wd_s[j], preferred_element_type=jnp.float32)
        r0 = pl.multiple_of(j * rows_per, 16)

        def ln_next(r):
            xr = pl.multiple_of(nxt * TM + r, 16)
            xn_s[1 - slot, pl.ds(r, 16), :] = _layernorm(x_s[pl.ds(xr, 16), :])
        _attention_rows(qkv_s, att_s, r0, rows_per, i * TM, ln_next)
        return c
    lax.fori_loop(0, NF, ffn_body, 0)

    def final(last):
        @pl.when(i == 0)
        def _():
            wo_copy().wait()

        @pl.when(i > 0)
        def _():
            for c in range(NOC):
                o_copy(i - 1, c).wait()

        if not last:
            qkv_s[NG:3 * NG, 0:HALO, :] = qkv_s[NG:3 * NG, TM:TM + HALO, :]

        att = att_s[...]
        row0 = pl.multiple_of(i * TM, TM)
        for c in range(NOC):
            cs = slice(c * OC, (c + 1) * OC)
            s = jnp.dot(att, wo_s[:, cs], preferred_element_type=jnp.float32)
            f = acc_s[:, cs]
            if not last:
                acc_s[:, cs] = jnp.zeros((TM, OC), jnp.float32)
            xcur = x_s[pl.ds(row0, TM), cs]
            o_s[:, cs] = (xcur.astype(jnp.float32) + s * _silu(f)).astype(jnp.bfloat16)
            o_copy(i, c).start()

    @pl.when(i < NT - 1)
    def _():
        final(False)
        qkv_cols(xn_s[1 - slot], 0, 3 * D)

    @pl.when(i == NT - 1)
    def _():
        final(True)
        for c in range(NOC):
            o_copy(i, c).wait()


@jax.jit
def pallas_recurrent_scan__sliding_local_dilated__swiglu_ffn__prompt_kernel(
    A_x, A_wqkv, A_wo, B_x, B_w_gate, B_w_up, B_w_down):
    x = A_x.reshape(S, D)
    hbm = pl.BlockSpec(memory_space=pl.ANY)
    bf = jnp.bfloat16
    out = pl.pallas_call(
        _kernel,
        grid=(NT,),
        in_specs=[hbm] * 6,
        out_specs=hbm,
        out_shape=jax.ShapeDtypeStruct((S, D), bf),
        scratch_shapes=[
            pltpu.VMEM((S, D), bf),
            pltpu.VMEM((D, 3 * D), bf),
            pltpu.VMEM((D, D), bf),
            pltpu.VMEM((NF, D, TF), bf),
            pltpu.VMEM((NF, D, TF), bf),
            pltpu.VMEM((NF, TF, D), bf),
            pltpu.VMEM((2, TM, D), bf),
            pltpu.VMEM((3 * NG, TM + HALO, 128), jnp.float32),
            pltpu.VMEM((TM, D), bf),
            pltpu.VMEM((TM, D), jnp.float32),
            pltpu.VMEM((TM, D), bf),
            pltpu.SemaphoreType.DMA((NSEM,)),
            pltpu.SemaphoreType.DMA((NOC,)),
        ],
        compiler_params=pltpu.CompilerParams(
            dimension_semantics=("arbitrary",),
            vmem_limit_bytes=100 * 1024 * 1024,
        ),
    )(x, A_wqkv, A_wo, B_w_gate, B_w_up, B_w_down)
    return out.reshape(1, S, D)
```

```python
import jax
import jax.numpy as jnp
from jax import lax
import jax.experimental.pallas as pl
import jax.experimental.pallas.tpu as pltpu

S, D, F = 2048, 1024, 3584
H, DH, W, DIL = 32, 32, 8, 2
HALO = 16
NG = D // 128

TM = 512
TF = 896
NT = S // TM
NF = F // TF
NOC = 4
OCH = tuple(range(0, D + 1, D // NOC))
XC = 4
XR = TM // XC
_QW = (128,256,768)
_QN = (2,2,3)
QLOOPS = []
_c, _n = 0, 0
for _w, _k in zip(_QW, _QN):
    QLOOPS.append((_w, _k, _c, _n))
    _c, _n = _c + _w * _k, _n + _k
assert _c == 3 * D
NQ = _n
LCH = (0,384,768,896,1024)

SEM_X0 = 0
SEM_X = SEM_X0 + XC
SEM_Q = SEM_X + NT
SEM_O = SEM_Q + NQ
SEM_G = SEM_O + 1
SEM_U = SEM_G + NF
SEM_D = SEM_U + NF
NSEM = SEM_D + NF


def _blk_transpose(arrs):
    shape = arrs[0].shape
    lane = lax.broadcasted_iota(jnp.int32, shape, 1)
    q = lane >> 2
    rolled = [arrs[0]] + [pltpu.roll(arrs[g], 4 * g, 1) for g in range(1, 8)]
    r = [rolled[(-m) % 8] for m in range(8)]
    for b in range(3):
        bit = (q & (1 << b)) != 0
        r = [jnp.where(bit, r[(j - (1 << b)) % 8], r[j]) for j in range(8)]
    return [r[0]] + [pltpu.roll(r[j], 128 - 4 * j, 1) for j in range(1, 8)]


def _attention_rows(qkv_s, att_s, r0, nrows, row_base, extra):
    lane = lax.broadcasted_iota(jnp.int32, (16, 128), 1)
    even = (lane & 1) == 0
    low2 = (lane & 2) == 0
    c_exp = (DH ** -0.5) * 1.4426950408889634
    for rb in range(nrows // 16):
        r = r0 + rb * 16
        for base in (NG, 2 * NG):
            t = _blk_transpose([qkv_s[base + g, pl.ds(r + HALO, 16), :] for g in range(NG)])
            for g in range(NG):
                qkv_s[base + g, pl.ds(r + HALO, 16), :] = t[g]
        qs = _blk_transpose([qkv_s[g, pl.ds(r + HALO, 16), :] for g in range(NG)])
        if rb == 0:
            grow = row_base + r + lax.broadcasted_iota(jnp.int32, (16, 128), 0)
        logits = []
        for w in range(W):
            p = None
            for g in range(NG):
                t = qs[g] * qkv_s[NG + g, pl.ds(r + HALO - DIL * w, 16), :]
                p = t if p is None else p + t
            y = p + jnp.where(even, pltpu.roll(p, 127, 1), pltpu.roll(p, 1, 1))
            z = y + jnp.where(low2, pltpu.roll(y, 126, 1), pltpu.roll(y, 2, 1))
            if w > 0 and rb == 0:
                z = jnp.where(grow >= DIL * w, z, -1e9 * DH ** 0.5)
            logits.append(z)
        m = logits[0]
        for w in range(1, W):
            m = jnp.maximum(m, logits[w])
        es = [jnp.exp2((l - m) * c_exp) for l in logits]
        den = es[0]
        for w in range(1, W):
            den = den + es[w]
        inv = pl.reciprocal(den, approx=True)
        inv = inv * (2.0 - den * inv)
        ps = [e * inv for e in es]
        outs = []
        for g in range(NG):
            o = None
            for w in range(W):
                t = ps[w] * qkv_s[2 * NG + g, pl.ds(r + HALO - DIL * w, 16), :]
                o = t if o is None else o + t
            outs.append(o)
        outs = _blk_transpose(outs)
        for g in range(NG):
            att_s[pl.ds(r, 16), g * 128:(g + 1) * 128] = outs[g].astype(jnp.bfloat16)
        extra(r)


def _silu(x):
    t = 0.5 * x
    return t + t * jnp.tanh(t)


def _layernorm(x):
    x = x.astype(jnp.float32)
    mean = jnp.mean(x, axis=-1, keepdims=True)
    xc = x - mean
    var = jnp.mean(xc * xc, axis=-1, keepdims=True)
    return (xc * lax.rsqrt(var + 1e-5)).astype(jnp.bfloat16)


def _kernel(x_hbm, wqkv_hbm, wo_hbm, wg_hbm, wu_hbm, wd_hbm, o_hbm,
            x_s, wqkv_s, wo_s, wg_s, wu_s, wd_s,
            xn_s, qkv_s, att_s, acc_s, o_s, sem, sem_out):
    i = pl.program_id(0)

    def x0_copy(c):
        return pltpu.make_async_copy(x_hbm.at[pl.ds(c * XR, XR), :], x_s.at[pl.ds(c * XR, XR), :], sem.at[SEM_X0 + c])

    def x_copy(t):
        return pltpu.make_async_copy(x_hbm.at[pl.ds(t * TM, TM), :], x_s.at[pl.ds(t * TM, TM), :], sem.at[SEM_X + t])

    def q_copy(lp, t):
        w, _, c0, n0 = lp
        return pltpu.make_async_copy(wqkv_hbm.at[:, pl.ds(c0 + t * w, w)], wqkv_s.at[:, pl.ds(c0 + t * w, w)], sem.at[SEM_Q + n0 + t])

    def wo_copy():
        return pltpu.make_async_copy(wo_hbm, wo_s, sem.at[SEM_O])

    def g_copy(j):
        return pltpu.make_async_copy(wg_hbm.at[:, pl.ds(j * TF, TF)], wg_s.at[j], sem.at[SEM_G + j])

    def u_copy(j):
        return pltpu.make_async_copy(wu_hbm.at[:, pl.ds(j * TF, TF)], wu_s.at[j], sem.at[SEM_U + j])

    def d_copy(j):
        return pltpu.make_async_copy(wd_hbm.at[pl.ds(j * TF, TF), :], wd_s.at[j], sem.at[SEM_D + j])

    def o_copy(t, c, ch):
        c0, n = ch[c], ch[c + 1] - ch[c]
        return pltpu.make_async_copy(o_s.at[:, pl.ds(c0, n)], o_hbm.at[pl.ds(t * TM, TM), pl.ds(c0, n)], sem_out.at[c])

    def qkv_cols(xn, c0, n):
        static = isinstance(c0, int)
        w = wqkv_s[:, c0:c0 + n] if static else wqkv_s[:, pl.ds(pl.multiple_of(c0, 128), n)]
        res = jnp.dot(xn, w, preferred_element_type=jnp.float32)
        g0 = c0 // 128
        for k in range(n // 128):
            qkv_s[g0 + k, HALO:HALO + TM, :] = res[:, k * 128:(k + 1) * 128]

    @pl.when(i == 0)
    def _():
        for c in range(XC):
            x0_copy(c).start()
        for lp in QLOOPS:
            for t in range(lp[1]):
                q_copy(lp, t).start()
        for jj in range(NF):
            g_copy(jj).start()
            u_copy(jj).start()
            d_copy(jj).start()
            if jj == 0:
                x_copy(1).start()
        wo_copy().start()
        for t in range(2, NT):
            x_copy(t).start()
        qkv_s[NG:3 * NG, 0:HALO, :] = jnp.zeros((2 * NG, HALO, 128), jnp.float32)

        def zero_acc(c, carry):
            acc_s[pl.ds(pl.multiple_of(c * 64, 64), 64), :] = jnp.zeros((64, D), jnp.float32)
            return carry
        lax.fori_loop(0, TM // 64, zero_acc, 0)

        def ln0(c, carry):
            r = pl.multiple_of(c * XR, XR)
            x0_copy(c).wait()
            xn_s[0, pl.ds(r, XR), :] = _layernorm(x_s[pl.ds(r, XR), :])
            return carry
        lax.fori_loop(0, XC, ln0, 0)

        for lp in QLOOPS:
            def q_body(t, carry, lp=lp):
                q_copy(lp, t).wait()
                qkv_cols(xn_s[0], lp[2] + t * lp[0], lp[0])
                return carry
            lax.fori_loop(0, lp[1], q_body, 0)

    nxt = jnp.minimum(i + 1, NT - 1)
    slot = i % 2
    rows_per = TM // NF

    def ffn_body(j, c):
        @pl.when(i == 0)
        def _():
            g_copy(j).wait()
            u_copy(j).wait()
            d_copy(j).wait()

        @pl.when(jnp.logical_and(i < NT - 1, j == 0))
        def _():
            x_copy(nxt).wait()

        xn = xn_s[slot]
        g = jnp.dot(xn, wg_s[j], preferred_element_type=jnp.float32)
        u = jnp.dot(xn, wu_s[j], preferred_element_type=jnp.float32)
        h = (_silu(g) * u).astype(jnp.bfloat16)
        acc_s[...] += jnp.dot(h, wd_s[j], preferred_element_type=jnp.float32)
        r0 = pl.multiple_of(j * rows_per, 16)

        def ln_next(r):
            xr = pl.multiple_of(nxt * TM + r, 16)
            xn_s[1 - slot, pl.ds(r, 16), :] = _layernorm(x_s[pl.ds(xr, 16), :])
        _attention_rows(qkv_s, att_s, r0, rows_per, i * TM, ln_next)
        return c
    lax.fori_loop(0, NF, ffn_body, 0)

    def final(last):
        @pl.when(i == 0)
        def _():
            wo_copy().wait()

        @pl.when(i > 0)
        def _():
            for c in range(NOC):
                o_copy(i - 1, c, OCH).wait()

        if not last:
            qkv_s[NG:3 * NG, 0:HALO, :] = qkv_s[NG:3 * NG, TM:TM + HALO, :]

        att = att_s[...]
        row0 = pl.multiple_of(i * TM, TM)
        ch = LCH if last else OCH
        for c in range(len(ch) - 1):
            cs = slice(ch[c], ch[c + 1])
            s = jnp.dot(att, wo_s[:, cs], preferred_element_type=jnp.float32)
            f = acc_s[:, cs]
            if not last:
                acc_s[:, cs] = jnp.zeros((TM, ch[c + 1] - ch[c]), jnp.float32)
            xcur = x_s[pl.ds(row0, TM), cs]
            o_s[:, cs] = (xcur.astype(jnp.float32) + s * _silu(f)).astype(jnp.bfloat16)
            o_copy(i, c, ch).start()

    @pl.when(i < NT - 1)
    def _():
        final(False)
        qkv_cols(xn_s[1 - slot], 0, 3 * D)

    @pl.when(i == NT - 1)
    def _():
        final(True)
        for c in range(len(LCH) - 1):
            o_copy(i, c, LCH).wait()


@jax.jit
def pallas_recurrent_scan__sliding_local_dilated__swiglu_ffn__prompt_kernel(
    A_x, A_wqkv, A_wo, B_x, B_w_gate, B_w_up, B_w_down):
    x = A_x.reshape(S, D)
    hbm = pl.BlockSpec(memory_space=pl.ANY)
    bf = jnp.bfloat16
    out = pl.pallas_call(
        _kernel,
        grid=(NT,),
        in_specs=[hbm] * 6,
        out_specs=hbm,
        out_shape=jax.ShapeDtypeStruct((S, D), bf),
        scratch_shapes=[
            pltpu.VMEM((S, D), bf),
            pltpu.VMEM((D, 3 * D), bf),
            pltpu.VMEM((D, D), bf),
            pltpu.VMEM((NF, D, TF), bf),
            pltpu.VMEM((NF, D, TF), bf),
            pltpu.VMEM((NF, TF, D), bf),
            pltpu.VMEM((2, TM, D), bf),
            pltpu.VMEM((3 * NG, TM + HALO, 128), jnp.float32),
            pltpu.VMEM((TM, D), bf),
            pltpu.VMEM((TM, D), jnp.float32),
            pltpu.VMEM((TM, D), bf),
            pltpu.SemaphoreType.DMA((NSEM,)),
            pltpu.SemaphoreType.DMA((max(NOC, len(LCH) - 1),)),
        ],
        compiler_params=pltpu.CompilerParams(
            dimension_semantics=("arbitrary",),
            vmem_limit_bytes=100 * 1024 * 1024,
        ),
    )(x, A_wqkv, A_wo, B_w_gate, B_w_up, B_w_down)
    return out.reshape(1, S, D)
```

```python
import jax
import jax.numpy as jnp
from jax import lax
import jax.experimental.pallas as pl
import jax.experimental.pallas.tpu as pltpu

S, D, F = 2048, 1024, 3584
H, DH, W, DIL = 32, 32, 8, 2
HALO = 16
NG = D // 128

TM = 512
TF = 896
NT = S // TM
NF = F // TF
NOC = 4
OCH = tuple(range(0, D + 1, D // NOC))
XC = 2
XR = TM // XC
_QW = (128,256,768)
_QN = (2,2,3)
QLOOPS = []
_c, _n = 0, 0
for _w, _k in zip(_QW, _QN):
    QLOOPS.append((_w, _k, _c, _n))
    _c, _n = _c + _w * _k, _n + _k
assert _c == 3 * D
NQ = _n
LCH = (0,384,768,896,1024)

NSEM = 6
QSEM = ((0, 5), (1, 1), (3, 1))
SEM_X0 = 3
SEM_WO = 4
SEM_OUT = 5


def _blk_transpose(arrs):
    shape = arrs[0].shape
    lane = lax.broadcasted_iota(jnp.int32, shape, 1)
    q = lane >> 2
    rolled = [arrs[0]] + [pltpu.roll(arrs[g], 4 * g, 1) for g in range(1, 8)]
    r = [rolled[(-m) % 8] for m in range(8)]
    for b in range(3):
        bit = (q & (1 << b)) != 0
        r = [jnp.where(bit, r[(j - (1 << b)) % 8], r[j]) for j in range(8)]
    return [r[0]] + [pltpu.roll(r[j], 128 - 4 * j, 1) for j in range(1, 8)]


def _attention_rows(qkv_s, att_s, r0, nrows, row_base, extra):
    lane = lax.broadcasted_iota(jnp.int32, (16, 128), 1)
    even = (lane & 1) == 0
    low2 = (lane & 2) == 0
    c_exp = (DH ** -0.5) * 1.4426950408889634
    for rb in range(nrows // 16):
        r = r0 + rb * 16
        for base in (NG, 2 * NG):
            t = _blk_transpose([qkv_s[base + g, pl.ds(r + HALO, 16), :] for g in range(NG)])
            for g in range(NG):
                qkv_s[base + g, pl.ds(r + HALO, 16), :] = t[g]
        qs = _blk_transpose([qkv_s[g, pl.ds(r + HALO, 16), :] for g in range(NG)])
        if rb == 0:
            grow = row_base + r + lax.broadcasted_iota(jnp.int32, (16, 128), 0)
        logits = []
        for w in range(W):
            p = None
            for g in range(NG):
                t = qs[g] * qkv_s[NG + g, pl.ds(r + HALO - DIL * w, 16), :]
                p = t if p is None else p + t
            y = p + jnp.where(even, pltpu.roll(p, 127, 1), pltpu.roll(p, 1, 1))
            z = y + jnp.where(low2, pltpu.roll(y, 126, 1), pltpu.roll(y, 2, 1))
            if w > 0 and rb == 0:
                z = jnp.where(grow >= DIL * w, z, -1e9 * DH ** 0.5)
            logits.append(z)
        m = logits[0]
        for w in range(1, W):
            m = jnp.maximum(m, logits[w])
        es = [jnp.exp2((l - m) * c_exp) for l in logits]
        den = es[0]
        for w in range(1, W):
            den = den + es[w]
        inv = pl.reciprocal(den, approx=True)
        inv = inv * (2.0 - den * inv)
        ps = [e * inv for e in es]
        outs = []
        for g in range(NG):
            o = None
            for w in range(W):
                t = ps[w] * qkv_s[2 * NG + g, pl.ds(r + HALO - DIL * w, 16), :]
                o = t if o is None else o + t
            outs.append(o)
        outs = _blk_transpose(outs)
        for g in range(NG):
            att_s[pl.ds(r, 16), g * 128:(g + 1) * 128] = outs[g].astype(jnp.bfloat16)
        extra(r)


def _silu(x):
    t = 0.5 * x
    return t + t * jnp.tanh(t)


def _layernorm(x):
    x = x.astype(jnp.float32)
    mean = jnp.mean(x, axis=-1, keepdims=True)
    xc = x - mean
    var = jnp.mean(xc * xc, axis=-1, keepdims=True)
    return (xc * lax.rsqrt(var + 1e-5)).astype(jnp.bfloat16)


def _kernel(x_hbm, wqkv_hbm, wo_hbm, wg_hbm, wu_hbm, wd_hbm, o_hbm,
            x_s, wqkv_s, wo_s, wg_s, wu_s, wd_s,
            xn_s, qkv_s, att_s, acc_s, o_s, sem):
    i = pl.program_id(0)

    def x0_copy(c):
        return pltpu.make_async_copy(x_hbm.at[pl.ds(c * XR, XR), :], x_s.at[pl.ds(c * XR, XR), :], sem.at[SEM_X0 + c])

    def ffn_sem(j):
        return sem.at[j]

    def x_copy(t):
        return pltpu.make_async_copy(x_hbm.at[pl.ds(t * TM, TM), :], x_s.at[pl.ds(t * TM, TM), :],
                                     ffn_sem(0) if t == 1 else sem.at[SEM_WO])

    def q_copy(n, t):
        w, _, c0, _ = QLOOPS[n]
        return pltpu.make_async_copy(wqkv_hbm.at[:, pl.ds(c0 + t * w, w)], wqkv_s.at[:, pl.ds(c0 + t * w, w)], sem.at[QSEM[n][0] + t * QSEM[n][1]])

    def wo_copy():
        return pltpu.make_async_copy(wo_hbm, wo_s, sem.at[SEM_WO])

    def g_copy(j):
        return pltpu.make_async_copy(wg_hbm.at[:, pl.ds(j * TF, TF)], wg_s.at[j], ffn_sem(j))

    def u_copy(j):
        return pltpu.make_async_copy(wu_hbm.at[:, pl.ds(j * TF, TF)], wu_s.at[j], ffn_sem(j))

    def d_copy(j):
        return pltpu.make_async_copy(wd_hbm.at[pl.ds(j * TF, TF), :], wd_s.at[j], ffn_sem(j))

    def o_copy(t, c, ch):
        c0, n = ch[c], ch[c + 1] - ch[c]
        return pltpu.make_async_copy(o_s.at[:, pl.ds(c0, n)], o_hbm.at[pl.ds(t * TM, TM), pl.ds(c0, n)], sem.at[SEM_OUT])

    def ffn_start(jj):
        g_copy(jj).start()
        u_copy(jj).start()
        d_copy(jj).start()

    def qkv_cols(xn, c0, n):
        static = isinstance(c0, int)
        w = wqkv_s[:, c0:c0 + n] if static else wqkv_s[:, pl.ds(pl.multiple_of(c0, 128), n)]
        res = jnp.dot(xn, w, preferred_element_type=jnp.float32)
        g0 = c0 // 128
        for k in range(n // 128):
            qkv_s[g0 + k, HALO:HALO + TM, :] = res[:, k * 128:(k + 1) * 128]

    @pl.when(i == 0)
    def _():
        for c in range(XC):
            x0_copy(c).start()
        for n in range(2):
            for t in range(2):
                q_copy(n, t).start()
        qkv_s[NG:3 * NG, 0:HALO, :] = jnp.zeros((2 * NG, HALO, 128), jnp.float32)

        def zero_acc(c, carry):
            acc_s[pl.ds(pl.multiple_of(c * 64, 64), 64), :] = jnp.zeros((64, D), jnp.float32)
            return carry
        lax.fori_loop(0, TM // 64, zero_acc, 0)

        def ln0(c, carry):
            r = pl.multiple_of(c * XR, XR)
            x0_copy(c).wait()
            xn_s[0, pl.ds(r, XR), :] = _layernorm(x_s[pl.ds(r, XR), :])
            return carry
        lax.fori_loop(0, XC, ln0, 0)

        def q_loop(n):
            w, cnt, c0, _ = QLOOPS[n]

            def q_body(t, carry):
                q_copy(n, t).wait()
                qkv_cols(xn_s[0], c0 + t * w, w)
                return carry
            lax.fori_loop(0, cnt, q_body, 0)

        q_copy(2, 0).start()
        q_copy(2, 1).start()
        q_loop(0)
        q_copy(2, 2).start()
        ffn_start(0)
        x_copy(1).start()
        q_loop(1)
        ffn_start(1)
        ffn_start(2)
        q_loop(2)
        ffn_start(3)
        wo_copy().start()
        for t in range(2, NT):
            x_copy(t).start()

    nxt = jnp.minimum(i + 1, NT - 1)
    slot = i % 2
    rows_per = TM // NF

    def ffn_body(j, c):
        @pl.when(i == 0)
        def _():
            g_copy(j).wait()
            u_copy(j).wait()
            d_copy(j).wait()

        @pl.when(jnp.logical_and(i == 0, j == 0))
        def _():
            x_copy(1).wait()

        xn = xn_s[slot]
        g = jnp.dot(xn, wg_s[j], preferred_element_type=jnp.float32)
        u = jnp.dot(xn, wu_s[j], preferred_element_type=jnp.float32)
        h = (_silu(g) * u).astype(jnp.bfloat16)
        acc_s[...] += jnp.dot(h, wd_s[j], preferred_element_type=jnp.float32)
        r0 = pl.multiple_of(j * rows_per, 16)

        def ln_next(r):
            xr = pl.multiple_of(nxt * TM + r, 16)
            xn_s[1 - slot, pl.ds(r, 16), :] = _layernorm(x_s[pl.ds(xr, 16), :])
        _attention_rows(qkv_s, att_s, r0, rows_per, i * TM, ln_next)
        return c
    lax.fori_loop(0, NF, ffn_body, 0)

    def final(last):
        @pl.when(i == 0)
        def _():
            wo_copy().wait()
            for t in range(2, NT):
                x_copy(t).wait()

        @pl.when(i > 0)
        def _():
            for c in range(NOC):
                o_copy(i - 1, c, OCH).wait()

        if not last:
            qkv_s[NG:3 * NG, 0:HALO, :] = qkv_s[NG:3 * NG, TM:TM + HALO, :]

        att = att_s[...]
        row0 = pl.multiple_of(i * TM, TM)
        ch = LCH if last else OCH
        for c in range(len(ch) - 1):
            cs = slice(ch[c], ch[c + 1])
            s = jnp.dot(att, wo_s[:, cs], preferred_element_type=jnp.float32)
            f = acc_s[:, cs]
            if not last:
                acc_s[:, cs] = jnp.zeros((TM, ch[c + 1] - ch[c]), jnp.float32)
            xcur = x_s[pl.ds(row0, TM), cs]
            o_s[:, cs] = (xcur.astype(jnp.float32) + s * _silu(f)).astype(jnp.bfloat16)
            o_copy(i, c, ch).start()

    @pl.when(i < NT - 1)
    def _():
        final(False)
        qkv_cols(xn_s[1 - slot], 0, 3 * D)

    @pl.when(i == NT - 1)
    def _():
        final(True)
        for c in range(len(LCH) - 1):
            o_copy(i, c, LCH).wait()


@jax.jit
def pallas_recurrent_scan__sliding_local_dilated__swiglu_ffn__prompt_kernel(
    A_x, A_wqkv, A_wo, B_x, B_w_gate, B_w_up, B_w_down):
    x = A_x.reshape(S, D)
    hbm = pl.BlockSpec(memory_space=pl.ANY)
    bf = jnp.bfloat16
    out = pl.pallas_call(
        _kernel,
        grid=(NT,),
        in_specs=[hbm] * 6,
        out_specs=hbm,
        out_shape=jax.ShapeDtypeStruct((S, D), bf),
        scratch_shapes=[
            pltpu.VMEM((S, D), bf),
            pltpu.VMEM((D, 3 * D), bf),
            pltpu.VMEM((D, D), bf),
            pltpu.VMEM((NF, D, TF), bf),
            pltpu.VMEM((NF, D, TF), bf),
            pltpu.VMEM((NF, TF, D), bf),
            pltpu.VMEM((2, TM, D), bf),
            pltpu.VMEM((3 * NG, TM + HALO, 128), jnp.float32),
            pltpu.VMEM((TM, D), bf),
            pltpu.VMEM((TM, D), jnp.float32),
            pltpu.VMEM((TM, D), bf),
            pltpu.SemaphoreType.DMA((NSEM,)),
        ],
        compiler_params=pltpu.CompilerParams(
            dimension_semantics=("arbitrary",),
            vmem_limit_bytes=100 * 1024 * 1024,
        ),
    )(x, A_wqkv, A_wo, B_w_gate, B_w_up, B_w_down)
    return out.reshape(1, S, D)
```

```python
import jax
import jax.numpy as jnp
from jax import lax
import jax.experimental.pallas as pl
import jax.experimental.pallas.tpu as pltpu

S, D, F = 2048, 1024, 3584
H, DH, W, DIL = 32, 32, 8, 2
HALO = 16
NG = D // 128

TM = 512
TF = 896
NT = S // TM
NF = F // TF
XC = 2
XR = TM // XC
OCH = (0, 256, 512, 768, 1024)
LCH = (0, 384, 768, 896, 1024)
QLOOPS = ((128, 2, 0), (256, 2, 256), (768, 3, 768))

NSEM = 6
QSEM = ((0, 5), (1, 1), (3, 1))
SEM_X0 = 3
SEM_WO = 4
SEM_OUT = 5


def _blk_transpose(arrs):
    lane = lax.broadcasted_iota(jnp.int32, arrs[0].shape, 1)
    q = lane >> 2
    rolled = [arrs[0]] + [pltpu.roll(arrs[g], 4 * g, 1) for g in range(1, 8)]
    r = [rolled[(-m) % 8] for m in range(8)]
    for b in range(3):
        bit = (q & (1 << b)) != 0
        r = [jnp.where(bit, r[(j - (1 << b)) % 8], r[j]) for j in range(8)]
    return [r[0]] + [pltpu.roll(r[j], 128 - 4 * j, 1) for j in range(1, 8)]


def _attention_rows(qkv_s, att_s, r0, nrows, row_base, extra):
    lane = lax.broadcasted_iota(jnp.int32, (16, 128), 1)
    even = (lane & 1) == 0
    low2 = (lane & 2) == 0
    c_exp = (DH ** -0.5) * 1.4426950408889634
    for rb in range(nrows // 16):
        r = r0 + rb * 16
        for base in (NG, 2 * NG):
            t = _blk_transpose([qkv_s[base + g, pl.ds(r + HALO, 16), :] for g in range(NG)])
            for g in range(NG):
                qkv_s[base + g, pl.ds(r + HALO, 16), :] = t[g]
        qs = _blk_transpose([qkv_s[g, pl.ds(r + HALO, 16), :] for g in range(NG)])
        if rb == 0:
            grow = row_base + r + lax.broadcasted_iota(jnp.int32, (16, 128), 0)
        logits = []
        for w in range(W):
            p = None
            for g in range(NG):
                t = qs[g] * qkv_s[NG + g, pl.ds(r + HALO - DIL * w, 16), :]
                p = t if p is None else p + t
            y = p + jnp.where(even, pltpu.roll(p, 127, 1), pltpu.roll(p, 1, 1))
            z = y + jnp.where(low2, pltpu.roll(y, 126, 1), pltpu.roll(y, 2, 1))
            if w > 0 and rb == 0:
                z = jnp.where(grow >= DIL * w, z, -1e9 * DH ** 0.5)
            logits.append(z)
        m = logits[0]
        for w in range(1, W):
            m = jnp.maximum(m, logits[w])
        es = [jnp.exp2((l - m) * c_exp) for l in logits]
        den = es[0]
        for w in range(1, W):
            den = den + es[w]
        inv = pl.reciprocal(den, approx=True)
        inv = inv * (2.0 - den * inv)
        ps = [e * inv for e in es]
        outs = []
        for g in range(NG):
            o = None
            for w in range(W):
                t = ps[w] * qkv_s[2 * NG + g, pl.ds(r + HALO - DIL * w, 16), :]
                o = t if o is None else o + t
            outs.append(o)
        outs = _blk_transpose(outs)
        for g in range(NG):
            att_s[pl.ds(r, 16), g * 128:(g + 1) * 128] = outs[g].astype(jnp.bfloat16)
        extra(r)


def _silu(x):
    t = 0.5 * x
    return t + t * jnp.tanh(t)


def _layernorm(x):
    x = x.astype(jnp.float32)
    mean = jnp.mean(x, axis=-1, keepdims=True)
    xc = x - mean
    var = jnp.mean(xc * xc, axis=-1, keepdims=True)
    return (xc * lax.rsqrt(var + 1e-5)).astype(jnp.bfloat16)


def _kernel(x_hbm, wqkv_hbm, wo_hbm, wg_hbm, wu_hbm, wd_hbm, o_hbm,
            x_s, wqkv_s, wo_s, wg_s, wu_s, wd_s,
            xn_s, qkv_s, att_s, acc_s, o_s, sem):
    i = pl.program_id(0)

    def x0_copy(c):
        rows = pl.ds(c * XR, XR)
        return pltpu.make_async_copy(x_hbm.at[rows, :], x_s.at[rows, :], sem.at[SEM_X0 + c])

    def x_copy(t):
        rows = pl.ds(t * TM, TM)
        return pltpu.make_async_copy(x_hbm.at[rows, :], x_s.at[rows, :], sem.at[0 if t == 1 else SEM_WO])

    def q_copy(n, t):
        w, _, c0 = QLOOPS[n]
        cols = pl.ds(c0 + t * w, w)
        return pltpu.make_async_copy(wqkv_hbm.at[:, cols], wqkv_s.at[:, cols],
                                     sem.at[QSEM[n][0] + t * QSEM[n][1]])

    def wo_copy():
        return pltpu.make_async_copy(wo_hbm, wo_s, sem.at[SEM_WO])

    def g_copy(j):
        return pltpu.make_async_copy(wg_hbm.at[:, pl.ds(j * TF, TF)], wg_s.at[j], sem.at[j])

    def u_copy(j):
        return pltpu.make_async_copy(wu_hbm.at[:, pl.ds(j * TF, TF)], wu_s.at[j], sem.at[j])

    def d_copy(j):
        return pltpu.make_async_copy(wd_hbm.at[pl.ds(j * TF, TF), :], wd_s.at[j], sem.at[j])

    def o_copy(t, c, ch):
        cols = pl.ds(ch[c], ch[c + 1] - ch[c])
        return pltpu.make_async_copy(o_s.at[:, cols], o_hbm.at[pl.ds(t * TM, TM), cols], sem.at[SEM_OUT])

    def ffn_start(jj):
        g_copy(jj).start()
        u_copy(jj).start()
        d_copy(jj).start()

    def qkv_cols(xn, c0, n):
        static = isinstance(c0, int)
        w = wqkv_s[:, c0:c0 + n] if static else wqkv_s[:, pl.ds(pl.multiple_of(c0, 128), n)]
        res = jnp.dot(xn, w, preferred_element_type=jnp.float32)
        g0 = c0 // 128
        for k in range(n // 128):
            qkv_s[g0 + k, HALO:HALO + TM, :] = res[:, k * 128:(k + 1) * 128]

    @pl.when(i == 0)
    def _():
        for c in range(XC):
            x0_copy(c).start()
        for n in range(2):
            for t in range(2):
                q_copy(n, t).start()
        qkv_s[NG:3 * NG, 0:HALO, :] = jnp.zeros((2 * NG, HALO, 128), jnp.float32)

        def zero_acc(c, carry):
            acc_s[pl.ds(pl.multiple_of(c * 64, 64), 64), :] = jnp.zeros((64, D), jnp.float32)
            return carry
        lax.fori_loop(0, TM // 64, zero_acc, 0)

        def ln0(c, carry):
            r = pl.multiple_of(c * XR, XR)
            x0_copy(c).wait()
            xn_s[0, pl.ds(r, XR), :] = _layernorm(x_s[pl.ds(r, XR), :])
            return carry
        lax.fori_loop(0, XC, ln0, 0)

        def q_loop(n):
            w, cnt, c0 = QLOOPS[n]

            def q_body(t, carry):
                q_copy(n, t).wait()
                qkv_cols(xn_s[0], c0 + t * w, w)
                return carry
            lax.fori_loop(0, cnt, q_body, 0)

        q_copy(2, 0).start()
        q_copy(2, 1).start()
        q_loop(0)
        q_copy(2, 2).start()
        ffn_start(0)
        x_copy(1).start()
        q_loop(1)
        ffn_start(1)
        ffn_start(2)
        q_loop(2)
        ffn_start(3)
        wo_copy().start()
        for t in range(2, NT):
            x_copy(t).start()

    nxt = jnp.minimum(i + 1, NT - 1)
    slot = i % 2
    rows_per = TM // NF

    def ffn_body(j, c):
        @pl.when(i == 0)
        def _():
            g_copy(j).wait()
            u_copy(j).wait()
            d_copy(j).wait()

        @pl.when(jnp.logical_and(i == 0, j == 0))
        def _():
            x_copy(1).wait()

        xn = xn_s[slot]
        g = jnp.dot(xn, wg_s[j], preferred_element_type=jnp.float32)
        u = jnp.dot(xn, wu_s[j], preferred_element_type=jnp.float32)
        h = (_silu(g) * u).astype(jnp.bfloat16)
        acc_s[...] += jnp.dot(h, wd_s[j], preferred_element_type=jnp.float32)
        r0 = pl.multiple_of(j * rows_per, 16)

        def ln_next(r):
            xr = pl.multiple_of(nxt * TM + r, 16)
            xn_s[1 - slot, pl.ds(r, 16), :] = _layernorm(x_s[pl.ds(xr, 16), :])
        _attention_rows(qkv_s, att_s, r0, rows_per, i * TM, ln_next)
        return c
    lax.fori_loop(0, NF, ffn_body, 0)

    def final(last):
        @pl.when(i == 0)
        def _():
            wo_copy().wait()
            for t in range(2, NT):
                x_copy(t).wait()

        @pl.when(i > 0)
        def _():
            for c in range(len(OCH) - 1):
                o_copy(i - 1, c, OCH).wait()

        if not last:
            qkv_s[NG:3 * NG, 0:HALO, :] = qkv_s[NG:3 * NG, TM:TM + HALO, :]

        att = att_s[...]
        row0 = pl.multiple_of(i * TM, TM)
        ch = LCH if last else OCH
        for c in range(len(ch) - 1):
            cs = slice(ch[c], ch[c + 1])
            s = jnp.dot(att, wo_s[:, cs], preferred_element_type=jnp.float32)
            f = acc_s[:, cs]
            if not last:
                acc_s[:, cs] = jnp.zeros((TM, ch[c + 1] - ch[c]), jnp.float32)
            xcur = x_s[pl.ds(row0, TM), cs]
            o_s[:, cs] = (xcur.astype(jnp.float32) + s * _silu(f)).astype(jnp.bfloat16)
            o_copy(i, c, ch).start()

    @pl.when(i < NT - 1)
    def _():
        final(False)
        qkv_cols(xn_s[1 - slot], 0, 3 * D)

    @pl.when(i == NT - 1)
    def _():
        final(True)
        for c in range(len(LCH) - 1):
            o_copy(i, c, LCH).wait()


@jax.jit
def pallas_recurrent_scan__sliding_local_dilated__swiglu_ffn__prompt_kernel(
    A_x: jax.Array,
    A_wqkv: jax.Array,
    A_wo: jax.Array,
    B_x: jax.Array,
    B_w_gate: jax.Array,
    B_w_up: jax.Array,
    B_w_down: jax.Array,
):
    del B_x
    x = A_x.reshape(S, D)
    hbm = pl.BlockSpec(memory_space=pl.ANY)
    bf = jnp.bfloat16
    out = pl.pallas_call(
        _kernel,
        grid=(NT,),
        in_specs=[hbm] * 6,
        out_specs=hbm,
        out_shape=jax.ShapeDtypeStruct((S, D), bf),
        scratch_shapes=[
            pltpu.VMEM((S, D), bf),
            pltpu.VMEM((D, 3 * D), bf),
            pltpu.VMEM((D, D), bf),
            pltpu.VMEM((NF, D, TF), bf),
            pltpu.VMEM((NF, D, TF), bf),
            pltpu.VMEM((NF, TF, D), bf),
            pltpu.VMEM((2, TM, D), bf),
            pltpu.VMEM((3 * NG, TM + HALO, 128), jnp.float32),
            pltpu.VMEM((TM, D), bf),
            pltpu.VMEM((TM, D), jnp.float32),
            pltpu.VMEM((TM, D), bf),
            pltpu.SemaphoreType.DMA((NSEM,)),
        ],
        compiler_params=pltpu.CompilerParams(
            dimension_semantics=("arbitrary",),
            vmem_limit_bytes=100 * 1024 * 1024,
        ),
    )(x, A_wqkv, A_wo, B_w_gate, B_w_up, B_w_down)
    return out.reshape(1, S, D)
```
